```python
import jax
import jax.numpy as jnp

def _softmax(x, axis=-1):
    return jax.nn.softmax(x, axis=axis)
def _gelu(x):
    return jax.nn.gelu(x, approximate=True)
def _silu(x):
    return jax.nn.silu(x)
def _sigmoid(x):
    return jax.nn.sigmoid(x)
def _layernorm(x, axis=-1, eps=1e-5):
    m = jnp.mean(x, axis=axis, keepdims=True)
    v = jnp.var(x, axis=axis, keepdims=True)
    return (x - m) / jnp.sqrt(v + eps)
def _scatter_add(tgt, idx, src, axis=0):
    return tgt.at[idx].add(src)
def _segment_sum(src, seg, n):
    return jax.ops.segment_sum(src, seg, n)
class _Rng:
    def __init__(self, key):
        self._k = key
    def _next(self):
        self._k, sub = jax.random.split(self._k)
        return sub
    def normal(self, shape):
        return jax.random.normal(self._next(), shape, dtype=jnp.bfloat16)
    def randint(self, lo, hi, shape):
        return jax.random.randint(self._next(), shape, lo, hi, dtype=jnp.int32)
    def uniform(self, shape, lo=0.0, hi=1.0):
        return jax.random.uniform(self._next(), shape, jnp.bfloat16, lo, hi)
    def permutation(self, n):
        return jax.random.permutation(self._next(), n)


kernel_name = 'standalone__standard_2d_1d_3d_conv__vision'

def setup_inputs():
    _rng = _Rng(jax.random.key(int.from_bytes(__import__("os").urandom(4), "little")))
    _w = (lambda a: (lambda t: t.astype(jnp.bfloat16) if jnp.issubdtype(t.dtype, jnp.floating) else t)(jnp.asarray(a)))
    H = W = 384
    C = 384
    K = 1
    return {
        "x": _w((lambda *s: _rng.normal(s) * 0.05)(1, H, W, C)),
        "w": _w((lambda *s: _rng.normal(s) * 0.05)(K, K, C, C)),
        "b": _w((lambda *s: _rng.normal(s) * 0.05)(C)),
    }

def reference(x, w, b):
    B, H, W, Cin = x.shape
    K = w.shape[0]
    pl = (K - 1) // 2
    pr = K // 2
    xp = jnp.pad(x, ((0, 0), (pl, pr), (pl, pr), (0, 0)))
    out = sum(
        jnp.einsum('bhwc,cd->bhwd', xp[:, i:i+H, j:j+W, :], w[i, j])
        for i in range(K) for j in range(K)
    )
    return out + b[None, None, None, :]
```

```python
import jax
import jax.numpy as jnp
from jax import lax
import jax.experimental.pallas as pl
import jax.experimental.pallas.tpu as pltpu

_PIECE_ROWS = 32
_NUM_CHUNKS = 32
_TILE_ROWS = 512


@jax.jit
def pallas_standalone__standard_2d_1d_3d_conv__vision_kernel(
    x: jax.Array,
    w: jax.Array,
    b: jax.Array,
):
    B, H, W, C = x.shape
    assert w.shape == (1, 1, C, C) and b.shape == (C,)
    M = B * H * W
    P, NB, TM = _PIECE_ROWS, _NUM_CHUNKS, _TILE_ROWS
    A = M // (P * NB)
    TA = TM // P
    assert A * P * NB == M and A % TA == 0
    NH = NB // 2

    def kernel(x_hbm, w_hbm, b_hbm, o_hbm, buf, w_vmem, b_vmem, rsem, wsem, csem):
        def read(j):
            return pltpu.make_async_copy(x_hbm.at[:, j], buf.at[j], rsem.at[j])

        def write(j):
            return pltpu.make_async_copy(buf.at[j], o_hbm.at[:, j], wsem.at[0])

        copy_w = pltpu.make_async_copy(w_hbm, w_vmem, csem.at[0])
        copy_b = pltpu.make_async_copy(b_hbm, b_vmem, csem.at[1])
        read(0).start()
        copy_w.start()
        copy_b.start()
        lax.fori_loop(1, NB, lambda j, _: read(j).start(), None)
        copy_w.wait()
        copy_b.wait()

        def compute(j):
            def tile(t, _):
                rows = pl.ds(pl.multiple_of(t * TA, TA), TA)
                xt = buf[j, rows].reshape(TM, C)
                acc = jnp.dot(xt, w_vmem[...], preferred_element_type=jnp.float32)
                bias = b_vmem[...].astype(jnp.float32).reshape(1, C)
                buf[j, rows] = (acc + bias).astype(buf.dtype).reshape(TA, P, C)

            lax.fori_loop(0, A // TA, tile, None)

        def stage_a(j, _):
            read(j).wait()
            compute(j)

        def stage_b(j, _):
            compute(j)
            write(j).start()

        lax.fori_loop(0, NH, stage_a, None)
        lax.fori_loop(NH, NB, lambda j, _: read(j).wait(), None)
        lax.fori_loop(0, NH, lambda j, _: write(j).start(), None)
        lax.fori_loop(NH, NB, stage_b, None)
        lax.fori_loop(0, NB, lambda j, _: write(j).wait(), None)

    out = pl.pallas_call(
        kernel,
        in_specs=[pl.BlockSpec(memory_space=pltpu.HBM)] * 3,
        out_specs=pl.BlockSpec(memory_space=pltpu.HBM),
        out_shape=jax.ShapeDtypeStruct((A, NB, P, C), x.dtype),
        scratch_shapes=[
            pltpu.VMEM((NB, A, P, C), x.dtype),
            pltpu.VMEM((C, C), w.dtype),
            pltpu.VMEM((C,), b.dtype),
            pltpu.SemaphoreType.DMA((NB,)),
            pltpu.SemaphoreType.DMA((1,)),
            pltpu.SemaphoreType.DMA((2,)),
        ],
        compiler_params=pltpu.CompilerParams(vmem_limit_bytes=127 * 2**20),
    )(x.reshape(A, NB, P, C), w.reshape(C, C), b)
    return out.reshape(B, H, W, C)
```

```python
import jax
import jax.numpy as jnp
from jax import lax
import jax.experimental.pallas as pl
import jax.experimental.pallas.tpu as pltpu

_LANES = 128
_HALF_ROWS = 32
_HALVES = 64
_READ_SLABS = (14, 22, 36)
_WRITE_SLABS = (36, 22, 14)


def _bounds(sizes):
    out = [0]
    for s in sizes:
        out.append(out[-1] + s)
    return out


@jax.jit
def pallas_standalone__standard_2d_1d_3d_conv__vision_kernel(
    x: jax.Array,
    w: jax.Array,
    b: jax.Array,
):
    B, H, W, C = x.shape
    assert C == 3 * _LANES and w.shape == (1, 1, C, C) and b.shape == (C,)
    assert x.dtype == jnp.bfloat16
    M = B * H * W
    period_rows = _HALVES * _HALF_ROWS
    num_periods = 3 * M // period_rows
    num_slabs = num_periods // 3
    slab_pixels = period_rows
    rb, wb = _bounds(_READ_SLABS), _bounds(_WRITE_SLABS)
    assert num_slabs * slab_pixels == M and rb[-1] == wb[-1] == num_slabs
    assert rb[-2] >= wb[1]
    num_reads = len(_READ_SLABS)

    def kernel(x_hbm, w_hbm, b_hbm, o_hbm, buf, w_vmem, b_vmem, rsem, wsem, csem):
        def read(lo, hi, i):
            s = pl.ds(lo, hi - lo)
            return pltpu.make_async_copy(x_hbm.at[s], buf.at[s], rsem.at[i])

        def write(g, half, n):
            s = (pl.ds(3 * wb[g], 3 * _WRITE_SLABS[g]), pl.ds(half, n))
            return pltpu.make_async_copy(buf.at[s], o_hbm.at[s], wsem.at[0])

        def for_each_write(g, op):
            op(write(g, 0, 1))
            lax.fori_loop(0, _HALVES // 2 - 1, lambda j, _: op(write(g, 2 * j + 1, 2)), None)
            op(write(g, _HALVES - 1, 1))

        reads = [
            read(3 * rb[i], min(3 * rb[i + 1], num_periods - 1), i) for i in range(num_reads)
        ]
        last_read = read(num_periods - 1, num_periods, num_reads)
        copy_w = pltpu.make_async_copy(w_hbm, w_vmem, csem.at[0])
        copy_b = pltpu.make_async_copy(b_hbm, b_vmem, csem.at[1])

        queue = [copy_w, copy_b, *reads, last_read]

        def issue(i, _):
            for k, copy in enumerate(queue):
                pl.when(i == k)(copy.start)

        lax.fori_loop(0, len(queue), issue, None)
        copy_w.wait()
        copy_b.wait()

        def compute(t):
            periods = pl.ds(3 * t, 3)
            v = buf[periods].reshape(3 * period_rows, _LANES)
            u = pltpu.bitcast(v, jnp.uint32).reshape(slab_pixels // 16, 3, 8, _LANES)
            u0, u1, u2 = u[:, 0], u[:, 1], u[:, 2]
            low = lax.broadcasted_iota(jnp.int32, u0.shape, 1) < 4
            blocks = (
                jnp.where(low, u0, u1),
                pltpu.roll(jnp.where(low, u2, u0), 4, 1),
                jnp.where(low, u1, u2),
            )
            xt = jnp.concatenate(
                [
                    pltpu.bitcast(blk.reshape(slab_pixels // 2, _LANES), buf.dtype)
                    for blk in blocks
                ],
                axis=1,
            )
            acc = jnp.dot(xt, w_vmem[...], preferred_element_type=jnp.float32)
            y = (acc + b_vmem[...].astype(jnp.float32).reshape(1, C)).astype(buf.dtype)
            y0, y1, y2 = (
                pltpu.bitcast(y[:, c * _LANES:(c + 1) * _LANES], jnp.uint32).reshape(u0.shape)
                for c in range(3)
            )
            y1 = pltpu.roll(y1, 4, 1)
            o = jnp.stack(
                [jnp.where(low, y0, y1), jnp.where(low, y2, y0), jnp.where(low, y1, y2)],
                axis=1,
            )
            o = pltpu.bitcast(o.reshape(3 * period_rows // 2, _LANES), buf.dtype)
            buf[periods] = o.reshape(3, _HALVES, _HALF_ROWS, _LANES)

        def step(t, _):
            for i in range(num_reads):
                if rb[i] < wb[1]:
                    pl.when(t == rb[i])(reads[i].wait)
            compute(t)
            for g in range(len(_WRITE_SLABS)):

                @pl.when(t == wb[g + 1] - 1)
                def _(g=g):
                    if g == 0:
                        for i in range(num_reads):
                            if rb[i] >= wb[1]:
                                reads[i].wait()
                    for_each_write(g, lambda copy: copy.start())
                    if g == 0:
                        last_read.wait()

        lax.fori_loop(0, num_slabs, step, None)
        for g in range(len(_WRITE_SLABS)):
            for_each_write(g, lambda copy: copy.wait())

    view = (num_periods, _HALVES, _HALF_ROWS, _LANES)
    x_view = x.reshape(M // 8, 8, 3, _LANES).transpose(0, 2, 1, 3).reshape(view)
    out = pl.pallas_call(
        kernel,
        in_specs=[pl.BlockSpec(memory_space=pltpu.HBM)] * 3,
        out_specs=pl.BlockSpec(memory_space=pltpu.HBM),
        out_shape=jax.ShapeDtypeStruct(view, x.dtype),
        scratch_shapes=[
            pltpu.VMEM(view, x.dtype),
            pltpu.VMEM((C, C), w.dtype),
            pltpu.VMEM((C,), b.dtype),
            pltpu.SemaphoreType.DMA((num_reads + 1,)),
            pltpu.SemaphoreType.DMA((1,)),
            pltpu.SemaphoreType.DMA((2,)),
        ],
        compiler_params=pltpu.CompilerParams(vmem_limit_bytes=127 * 2**20),
    )(x_view, w.reshape(C, C), b)
    return out.reshape(M // 8, 3, 8, _LANES).transpose(0, 2, 1, 3).reshape(B, H, W, C)
```

```python
import jax
import jax.numpy as jnp
from jax import lax
import jax.experimental.pallas as pl
import jax.experimental.pallas.tpu as pltpu

_LANES = 128
_HALF_ROWS = 32
_HALVES = 64
_READ_BOUNDS = (0, 8, 20, 36, 72)
_WRITE_BOUNDS = (0, 36, 54, 64, 72)


@jax.jit
def pallas_standalone__standard_2d_1d_3d_conv__vision_kernel(
    x: jax.Array,
    w: jax.Array,
    b: jax.Array,
):
    B, H, W, C = x.shape
    assert C == 3 * _LANES and w.shape == (1, 1, C, C) and b.shape == (C,)
    assert x.dtype == jnp.bfloat16
    M = B * H * W
    period_rows = _HALVES * _HALF_ROWS
    slab_pixels = period_rows
    num_slabs = M // slab_pixels
    num_periods = 3 * num_slabs
    assert num_slabs * slab_pixels == M and num_slabs % 72 == 0
    rb = [v * num_slabs // 72 for v in _READ_BOUNDS]
    wb = [v * num_slabs // 72 for v in _WRITE_BOUNDS]
    num_reads, num_groups = len(rb) - 1, len(wb) - 1
    assert rb[-2] == wb[1]

    def kernel(x_hbm, w_hbm, b_hbm, o_hbm, buf, w_vmem, b_vmem, rsem, wsem):
        def read(lo, hi, i):
            s = pl.ds(lo, hi - lo)
            return pltpu.make_async_copy(x_hbm.at[s], buf.at[s], rsem.at[i])

        def write(g, half, n):
            s = (pl.ds(3 * wb[g], 3 * (wb[g + 1] - wb[g])), pl.ds(half, n))
            return pltpu.make_async_copy(buf.at[s], o_hbm.at[s], wsem.at[0])

        def for_each_write(g, op):
            op(write(g, 0, 1))
            lax.fori_loop(0, _HALVES // 2 - 1, lambda j, _: op(write(g, 2 * j + 1, 2)), None)
            op(write(g, _HALVES - 1, 1))

        reads = [
            read(3 * rb[i], min(3 * rb[i + 1], num_periods - 1), i) for i in range(num_reads)
        ]
        last_read = read(num_periods - 1, num_periods, num_reads)
        first = [
            reads[0],
            pltpu.make_async_copy(w_hbm, w_vmem, rsem.at[0]),
            pltpu.make_async_copy(b_hbm, b_vmem, rsem.at[0]),
        ]
        for copy in first:
            copy.start()

        queue = [*reads[1:], last_read]

        def issue(i, _):
            for k, copy in enumerate(queue):
                pl.when(i == k)(copy.start)

        lax.fori_loop(0, len(queue), issue, None)
        for copy in first:
            copy.wait()

        def compute(t):
            periods = pl.ds(3 * t, 3)
            v = buf[periods].reshape(3 * period_rows, _LANES)
            u = pltpu.bitcast(v, jnp.uint32).reshape(slab_pixels // 16, 3, 8, _LANES)
            u0, u1, u2 = u[:, 0], u[:, 1], u[:, 2]
            low = lax.broadcasted_iota(jnp.int32, u0.shape, 1) < 4
            blocks = (
                jnp.where(low, u0, u1),
                pltpu.roll(jnp.where(low, u2, u0), 4, 1),
                jnp.where(low, u1, u2),
            )
            xt = jnp.concatenate(
                [
                    pltpu.bitcast(blk.reshape(slab_pixels // 2, _LANES), buf.dtype)
                    for blk in blocks
                ],
                axis=1,
            )
            acc = jnp.dot(xt, w_vmem[...], preferred_element_type=jnp.float32)
            y = (acc + b_vmem[...].astype(jnp.float32).reshape(1, C)).astype(buf.dtype)
            y0, y1, y2 = (
                pltpu.bitcast(y[:, c * _LANES:(c + 1) * _LANES], jnp.uint32).reshape(u0.shape)
                for c in range(3)
            )
            y1 = pltpu.roll(y1, 4, 1)
            o = jnp.stack(
                [jnp.where(low, y0, y1), jnp.where(low, y2, y0), jnp.where(low, y1, y2)],
                axis=1,
            )
            o = pltpu.bitcast(o.reshape(3 * period_rows // 2, _LANES), buf.dtype)
            buf[periods] = o.reshape(3, _HALVES, _HALF_ROWS, _LANES)

        def step(t, _):
            for i in range(1, num_reads - 1):
                pl.when(t == rb[i])(reads[i].wait)
            compute(t)
            for g in range(num_groups):

                @pl.when(t == wb[g + 1] - 1)
                def _(g=g):
                    if g == 0:
                        reads[-1].wait()
                    for_each_write(g, lambda copy: copy.start())
                    if g == 0:
                        last_read.wait()

        lax.fori_loop(0, num_slabs, step, None)
        for g in range(num_groups):
            for_each_write(g, lambda copy: copy.wait())

    view = (num_periods, _HALVES, _HALF_ROWS, _LANES)
    x_view = x.reshape(M // 8, 8, 3, _LANES).transpose(0, 2, 1, 3).reshape(view)
    out = pl.pallas_call(
        kernel,
        in_specs=[pl.BlockSpec(memory_space=pltpu.HBM)] * 3,
        out_specs=pl.BlockSpec(memory_space=pltpu.HBM),
        out_shape=jax.ShapeDtypeStruct(view, x.dtype),
        scratch_shapes=[
            pltpu.VMEM(view, x.dtype),
            pltpu.VMEM((C, C), w.dtype),
            pltpu.VMEM((C,), b.dtype),
            pltpu.SemaphoreType.DMA((num_reads + 1,)),
            pltpu.SemaphoreType.DMA((1,)),
        ],
        compiler_params=pltpu.CompilerParams(vmem_limit_bytes=120 * 2**20),
    )(x_view, w.reshape(C, C), b)
    return out.reshape(M // 8, 3, 8, _LANES).transpose(0, 2, 1, 3).reshape(B, H, W, C)
```
